```python
import jax
import jax.numpy as jnp

def _softmax(x, axis=-1):
    return jax.nn.softmax(x, axis=axis)
def _gelu(x):
    return jax.nn.gelu(x, approximate=True)
def _silu(x):
    return jax.nn.silu(x)
def _sigmoid(x):
    return jax.nn.sigmoid(x)
def _layernorm(x, axis=-1, eps=1e-5):
    m = jnp.mean(x, axis=axis, keepdims=True)
    v = jnp.var(x, axis=axis, keepdims=True)
    return (x - m) / jnp.sqrt(v + eps)
def _scatter_add(tgt, idx, src, axis=0):
    return tgt.at[idx].add(src)
def _segment_sum(src, seg, n):
    return jax.ops.segment_sum(src, seg, n)
class _Rng:
    def __init__(self, key):
        self._k = key
    def _next(self):
        self._k, sub = jax.random.split(self._k)
        return sub
    def normal(self, shape):
        return jax.random.normal(self._next(), shape, dtype=jnp.bfloat16)
    def randint(self, lo, hi, shape):
        return jax.random.randint(self._next(), shape, lo, hi, dtype=jnp.int32)
    def uniform(self, shape, lo=0.0, hi=1.0):
        return jax.random.uniform(self._next(), shape, jnp.bfloat16, lo, hi)
    def permutation(self, n):
        return jax.random.permutation(self._next(), n)


kernel_name = 'interleave_layers__sliding_block_cached__dense_activation_gelu__decode'

def _fwd_setup_inputs():
    _rng = _Rng(jax.random.key(int.from_bytes(__import__("os").urandom(4), "little")))
    _w = (lambda a: (lambda t: t.astype(jnp.bfloat16) if jnp.issubdtype(t.dtype, jnp.floating) else t)(jnp.asarray(a)))
    def _A_setup():
        B, Sq, D = 2, 1, 512
        Hq, Hkv, Sk, Dh = 32, 8, 32768, 128
        assert Hq % Hkv == 0, (Hq, Hkv)
        return {
            "x": _w((lambda *s: _rng.normal(s) * 0.05)(B, Sq, D)),
            "k_cache": _w((lambda *s: _rng.normal(s) * 0.05)(B, Hkv, Sk, Dh)),
            "v_cache": _w((lambda *s: _rng.normal(s) * 0.05)(B, Hkv, Sk, Dh)),
            "wq": _w((lambda *s: _rng.normal(s) * 0.05)(D, Hq * Dh) * (D ** -0.5)),
            "wo": _w((lambda *s: _rng.normal(s) * 0.05)(Hq * Dh, D) * ((Hq * Dh) ** -0.5)),
        }
    _A_in = _A_setup()

    def _B_setup():
        B, S, D, F = 2, 1, 512, 1792
        return {
            "x": _w((lambda *s: _rng.normal(s) * 0.05)(B, S, D)),
            "w1": _w((lambda *s: _rng.normal(s) * 0.05)(D, F) * (D ** -0.5)),
            "b1": _w((lambda *s: _rng.normal(s) * 0.05)(F) * 0.01),
            "w2": _w((lambda *s: _rng.normal(s) * 0.05)(F, D) * (F ** -0.5)),
            "b2": _w((lambda *s: _rng.normal(s) * 0.05)(D) * 0.01),
        }
    _B_in = _B_setup()

    return {
        "A_x": _A_in["x"],
        "A_k_cache": _A_in["k_cache"],
        "A_v_cache": _A_in["v_cache"],
        "A_wq": _A_in["wq"],
        "A_wo": _A_in["wo"],
        "B_x": _B_in["x"],
        "B_w1": _B_in["w1"],
        "B_b1": _B_in["b1"],
        "B_w2": _B_in["w2"],
        "B_b2": _B_in["b2"],
    }

def _fwd_reference(A_x, A_k_cache, A_v_cache, A_wq, A_wo, B_x, B_w1, B_b1, B_w2, B_b2):
    def _A_ref(x, k_cache, v_cache, wq, wo):
        B, Sq, D = x.shape
        Hq, Dh = 32, 128
        Hkv, Sk = k_cache.shape[1], k_cache.shape[2]
        W = min(4096, max(256, Sk // 4))
        rep = Hq // Hkv
        q = (lambda x, *d: x.transpose(*d))((x @ wq).reshape(B, Sq, Hq, Dh), 0, 2, 1, 3)
        k = jnp.repeat(k_cache[:, :, Sk - W:, :], rep, axis=1)
        v = jnp.repeat(v_cache[:, :, Sk - W:, :], rep, axis=1)
        scores = jnp.einsum("bhqd,bhkd->bhqk", q, k) * (Dh ** -0.5)
        p = _softmax(scores, axis=-1)
        o = jnp.einsum("bhqk,bhkd->bhqd", p, v)
        return (lambda x, *d: x.transpose(*d))(o, 0, 2, 1, 3).reshape(B, Sq, Hq * Dh) @ wo

    def _B_ref(x, w1, b1, w2, b2):
        h = jnp.einsum("bsd,df->bsf", x, w1) + b1
        h = _gelu(h)
        return jnp.einsum("bsf,fd->bsd", h, w2) + b2

    x = A_x
    x = x + _A_ref(_layernorm(x, axis=-1), A_k_cache, A_v_cache, A_wq, A_wo)
    x = x + _B_ref(_layernorm(x, axis=-1), B_w1, B_b1, B_w2, B_b2)
    x = x + _A_ref(_layernorm(x, axis=-1), A_k_cache, A_v_cache, A_wq, A_wo)
    x = x + _B_ref(_layernorm(x, axis=-1), B_w1, B_b1, B_w2, B_b2)
    return x


def setup_inputs():
    _inp = _fwd_setup_inputs()
    _gk = jax.random.fold_in(jax.random.key(int.from_bytes(__import__("os").urandom(4), "little")), 2**31 - 1)
    _shapes = [[2, 1, 512]]
    _dtypes = ['bfloat16']
    _gks = jax.random.split(_gk, len(_shapes))
    _gs = [jax.random.normal(k, s, dtype=jnp.dtype(d)) * 0.05 for k, s, d in zip(_gks, _shapes, _dtypes)]
    _inp["grad_out"] = _gs[0]
    return _inp

def reference(A_x, A_k_cache, A_v_cache, A_wq, A_wo, B_w1, B_b1, B_w2, B_b2, B_x, grad_out):
    _const = dict(B_x=B_x)
    def _f(*_d):
        return _fwd_reference(**{'A_x': _d[0], 'A_k_cache': _d[1], 'A_v_cache': _d[2], 'A_wq': _d[3], 'A_wo': _d[4], 'B_w1': _d[5], 'B_b1': _d[6], 'B_w2': _d[7], 'B_b2': _d[8], **_const})
    _out, _vjp = jax.vjp(_f, A_x, A_k_cache, A_v_cache, A_wq, A_wo, B_w1, B_b1, B_w2, B_b2)
    _grads = _vjp(grad_out)
    _out0 = jnp.asarray(_out)
    return (_out0, *[jnp.asarray(_g) for _g in _grads])
```

```python
import math

import jax
import jax.numpy as jnp
from jax import lax
import jax.experimental.pallas as pl
import jax.experimental.pallas.tpu as pltpu

_F32 = jnp.float32
_BF16 = jnp.bfloat16
_NT = (((1,), (1,)), ((), ()))
_TN = (((0,), (0,)), ((), ()))
_EPS = 1e-5
_GELU_C = math.sqrt(2.0 / math.pi)

_TILE = 16
_ZC = 4
_WC = 8
_DW_PIECE = 32768
_DW_NJ = 8


def _ln_fwd(x):
    m = jnp.mean(x, axis=-1, keepdims=True)
    xc = x - m
    v = jnp.mean(xc * xc, axis=-1, keepdims=True)
    r = lax.rsqrt(v + _EPS)
    return xc * r, r


def _ln_bwd(dy, y, r):
    return (dy - jnp.mean(dy, axis=-1, keepdims=True)
            - y * jnp.mean(dy * y, axis=-1, keepdims=True)) * r


@jax.jit
def pallas_interleave_layers__sliding_block_cached__dense_activation_gelu__decode_kernel(
    A_x: jax.Array,
    A_k_cache: jax.Array,
    A_v_cache: jax.Array,
    A_wq: jax.Array,
    A_wo: jax.Array,
    B_x: jax.Array,
    B_w1: jax.Array,
    B_b1: jax.Array,
    B_w2: jax.Array,
    B_b2: jax.Array,
    grad_out: jax.Array,
):
    B, SQ, D = A_x.shape
    assert SQ == 1
    _, HKV, SK, DH = A_k_cache.shape
    HQ = A_wq.shape[1] // DH
    F = B_w1.shape[1]
    W = min(4096, max(256, SK // 4))
    Z = SK - W
    REP = HQ // HKV
    NBH = B * HKV
    scale = DH ** -0.5
    assert REP == 4 and B == 2
    NJ = SK // W
    NC = W // (2 * _TILE)
    assert NJ * W == SK and NC % _ZC == 0 and NC % _WC == 0

    def kernel(x_hbm, g_hbm, b1_hbm, b2_hbm, k_hbm, v_hbm, wq_hbm, wo_hbm, w1_hbm, w2_hbm,
               out_hbm, dx_hbm, dk_hbm, dv_hbm, dwq_hbm, dwo_hbm, dw1_hbm, db1_hbm, dw2_hbm,
               db2_hbm,
               kbuf, vbuf, wq, wo, w1, w2, dwq_s, dwo_s, dw1_s, dw2_s, zbuf,
               q_s, do_s, o_s, dq_s, p_s, ds_s, flat_s,
               x_ref, g_ref, b1_ref, b2_ref, out_ref, dx_ref, db1_ref, db2_ref,
               sem_k, sem_v, sem_w, sem_z, sem_o, sem_s):

        def k_in(bh):
            return pltpu.make_async_copy(
                k_hbm.at[bh // HKV, bh % HKV, pl.ds(Z, W), :], kbuf.at[bh], sem_k.at[bh])

        def v_in(bh):
            return pltpu.make_async_copy(
                v_hbm.at[bh // HKV, bh % HKV, pl.ds(Z, W), :], vbuf.at[bh], sem_v.at[bh])

        w_in = [pltpu.make_async_copy(src, dst, sem_w.at[i]) for i, (src, dst) in enumerate(
            ((wq_hbm, wq), (wo_hbm, wo), (w1_hbm, w1), (w2_hbm, w2)))]
        s_in = [pltpu.make_async_copy(src, dst, sem_s.at[i]) for i, (src, dst) in enumerate(
            ((x_hbm, x_ref), (g_hbm, g_ref), (b1_hbm, b1_ref), (b2_hbm, b2_ref)))]

        z_out = [pltpu.make_async_copy(
            zbuf, o.at[:, pl.ds(0, NJ - 1), :, pl.ds(c * _ZC, _ZC)], sem_z.at[0])
            for c in range(NC // _ZC) for o in (dk_hbm, dv_hbm)]

        kbuf5 = kbuf.reshape(NBH, 2, NC, _TILE, DH)
        vbuf5 = vbuf.reshape(NBH, 2, NC, _TILE, DH)
        fin_out = [pltpu.make_async_copy(
            src.at[:, j2, pl.ds(c * _WC, _WC)], o.at[:, NJ - 1, j2, pl.ds(c * _WC, _WC)],
            sem_o.at[0])
            for j2 in range(2) for c in range(NC // _WC)
            for (src, o) in ((kbuf5, dk_hbm), (vbuf5, dv_hbm))]

        def dw_copies(src, dst):
            R, C = src.shape
            pr = max(_TILE, _DW_PIECE // (2 * C))
            nj = _DW_NJ if R % (_DW_NJ * pr) == 0 else _DW_NJ - 1
            assert R % (nj * pr) == 0 and pr % _TILE == 0
            nc = R // (nj * pr)
            s4 = src.reshape(nj, nc, pr, C)
            d4 = dst.reshape(nj, nc, pr, C)
            return [pltpu.make_async_copy(s4.at[:, c], d4.at[:, c], sem_o.at[0])
                    for c in range(nc)]

        for src, dst in ((dwq_s, dwq_hbm), (dwo_s, dwo_hbm), (dw1_s, dw1_hbm),
                         (dw2_s, dw2_hbm)):
            fin_out += dw_copies(src, dst)
        fin_out += [pltpu.make_async_copy(src, dst, sem_o.at[0]) for (src, dst) in (
            (out_ref, out_hbm), (dx_ref, dx_hbm), (db1_ref, db1_hbm), (db2_ref, db2_hbm))]

        for cp in s_in:
            cp.start()
        for cp in w_in:
            cp.start()
        for bh in range(NBH):
            k_in(bh).start()
            v_in(bh).start()
        zbuf[...] = jnp.zeros(zbuf.shape, zbuf.dtype)
        for cp in s_in:
            cp.wait()
        for cp in w_in:
            cp.wait()
        for bh in range(NBH):
            k_in(bh).wait()
            v_in(bh).wait()
            if bh == NBH - 2:
                for cp in z_out:
                    cp.start()

        def scatter_heads(full, dst, l):
            for b in range(B):
                for j in range(HQ):
                    dst[b * HKV + j // REP, pl.ds(l * REP + j % REP, 1), :] = (
                        full[b:b + 1, j * DH:(j + 1) * DH])

        def gather_heads(src, l):
            for b in range(B):
                for j in range(HQ):
                    flat_s[pl.ds(b, 1), pl.ds(j * DH, DH)] = (
                        src[b * HKV + j // REP, pl.ds(l * REP + j % REP, 1), :])
            return flat_s[pl.ds(0, B), :]

        def attn_fwd(l, ln):
            q = jnp.dot(ln.astype(_BF16), wq[...], preferred_element_type=_F32)
            scatter_heads(q, q_s, l)

            def body(bh, c):
                q4 = q_s[bh, pl.ds(l * REP, REP), :].astype(_BF16)
                s = lax.dot_general(q4, kbuf[bh], _NT, preferred_element_type=_F32) * scale
                m = jnp.max(s, axis=-1, keepdims=True)
                e = jnp.exp(s - m)
                p = e / jnp.sum(e, axis=-1, keepdims=True)
                p_s[bh, pl.ds(l * REP, REP), :] = p
                o_s[bh, pl.ds(l * REP, REP), :] = jnp.dot(
                    p.astype(_BF16), vbuf[bh], preferred_element_type=_F32)
                return c

            lax.fori_loop(0, NBH, body, 0)
            o = gather_heads(o_s, l)
            return o, jnp.dot(o.astype(_BF16), wo[...], preferred_element_type=_F32)

        def attn_bwd(l, dy, last):
            do = lax.dot_general(dy.astype(_BF16), wo[...], _NT, preferred_element_type=_F32)
            scatter_heads(do, do_s, l)

            def body(bh, c):
                do4 = do_s[bh, pl.ds(l * REP, REP), :].astype(_BF16)
                dp = lax.dot_general(do4, vbuf[bh], _NT, preferred_element_type=_F32)
                p = p_s[bh, pl.ds(l * REP, REP), :]
                ds = p * (dp - jnp.sum(p * dp, axis=-1, keepdims=True)) * scale
                ds_s[bh, pl.ds(l * REP, REP), :] = ds
                dq_s[bh, pl.ds(l * REP, REP), :] = jnp.dot(
                    ds.astype(_BF16), kbuf[bh], preferred_element_type=_F32)
                if last:
                    kbuf[bh] = lax.dot_general(
                        ds_s[bh].astype(_BF16), q_s[bh].astype(_BF16), _TN,
                        preferred_element_type=_F32).astype(_BF16)
                    vbuf[bh] = lax.dot_general(
                        p_s[bh].astype(_BF16), do_s[bh].astype(_BF16), _TN,
                        preferred_element_type=_F32).astype(_BF16)
                return c

            lax.fori_loop(0, NBH, body, 0)
            return gather_heads(dq_s, l)

        b1 = b1_ref[...].astype(_F32).reshape(1, F)
        b2 = b2_ref[...].astype(_F32).reshape(1, D)

        def mlp_fwd(ln):
            h = jnp.dot(ln.astype(_BF16), w1[...], preferred_element_type=_F32) + b1
            t = jnp.tanh(_GELU_C * (h + 0.044715 * (h * h * h)))
            g = 0.5 * h * (1.0 + t)
            y = jnp.dot(g.astype(_BF16), w2[...], preferred_element_type=_F32) + b2
            return h, t, g, y

        def mlp_bwd(dy, h, t):
            dg = lax.dot_general(dy.astype(_BF16), w2[...], _NT, preferred_element_type=_F32)
            dgelu = 0.5 * (1.0 + t) + 0.5 * h * (1.0 - t * t) * _GELU_C * (
                1.0 + 3.0 * 0.044715 * (h * h))
            dh = dg * dgelu
            dln = lax.dot_general(dh.astype(_BF16), w1[...], _NT, preferred_element_type=_F32)
            return dh, dln

        x0 = x_ref[...].astype(_F32)
        ln1, r1 = _ln_fwd(x0)
        o1, a1 = attn_fwd(0, ln1)
        x1 = x0 + a1
        ln2, r2 = _ln_fwd(x1)
        h2, t2, g2, y2 = mlp_fwd(ln2)
        x2 = x1 + y2
        ln3, r3 = _ln_fwd(x2)
        o3, a3 = attn_fwd(1, ln3)
        x3 = x2 + a3
        ln4, r4 = _ln_fwd(x3)
        h4, t4, g4, y4 = mlp_fwd(ln4)
        x4 = x3 + y4
        out_ref[...] = x4.astype(out_ref.dtype)

        dx4 = g_ref[...].astype(_F32)
        dh4, dln4 = mlp_bwd(dx4, h4, t4)
        dx3 = dx4 + _ln_bwd(dln4, ln4, r4)
        dq3 = attn_bwd(1, dx3, False)
        dln3 = lax.dot_general(dq3.astype(_BF16), wq[...], _NT, preferred_element_type=_F32)
        dx2 = dx3 + _ln_bwd(dln3, ln3, r3)
        dh2, dln2 = mlp_bwd(dx2, h2, t2)
        dx1 = dx2 + _ln_bwd(dln2, ln2, r2)
        dq1 = attn_bwd(0, dx1, True)
        dln1 = lax.dot_general(dq1.astype(_BF16), wq[...], _NT, preferred_element_type=_F32)
        dx0 = dx1 + _ln_bwd(dln1, ln1, r1)
        dx_ref[...] = dx0.astype(dx_ref.dtype)

        def stack(a, b):
            return jnp.concatenate([a, b], axis=0).astype(_BF16)

        def wgrad(a, bmat, dst, n_chunks):
            n = bmat.shape[1] // n_chunks
            for c in range(n_chunks):
                dst[:, pl.ds(c * n, n)] = lax.dot_general(
                    a, bmat[:, c * n:(c + 1) * n], _TN,
                    preferred_element_type=_F32).astype(dst.dtype)

        wgrad(stack(ln2, ln4), stack(dh2, dh4), dw1_s, 2)
        wgrad(stack(g2, g4), stack(dx2, dx4), dw2_s, 2)
        wgrad(stack(o1, o3), stack(dx1, dx3), dwo_s, 4)
        wgrad(stack(ln1, ln3), stack(dq1, dq3), dwq_s, 4)
        db1_ref[...] = jnp.sum(dh2 + dh4, axis=0).astype(db1_ref.dtype)
        db2_ref[...] = jnp.sum(dx2 + dx4, axis=0).astype(db2_ref.dtype)

        for cp in fin_out:
            cp.start()
        for cp in z_out:
            cp.wait()
        for cp in fin_out:
            cp.wait()

    hbm = pl.BlockSpec(memory_space=pl.ANY)
    cache_view = (NBH, NJ, 2, NC, _TILE, DH)
    out_shape = (
        jax.ShapeDtypeStruct((B, D), _BF16),
        jax.ShapeDtypeStruct((B, D), _BF16),
        jax.ShapeDtypeStruct(cache_view, _BF16),
        jax.ShapeDtypeStruct(cache_view, _BF16),
        jax.ShapeDtypeStruct(A_wq.shape, _BF16),
        jax.ShapeDtypeStruct(A_wo.shape, _BF16),
        jax.ShapeDtypeStruct(B_w1.shape, _BF16),
        jax.ShapeDtypeStruct(B_b1.shape, _BF16),
        jax.ShapeDtypeStruct(B_w2.shape, _BF16),
        jax.ShapeDtypeStruct(B_b2.shape, _BF16),
    )
    outs = pl.pallas_call(
        kernel,
        out_shape=out_shape,
        in_specs=[hbm] * 10,
        out_specs=(hbm,) * 10,
        scratch_shapes=[
            pltpu.VMEM((NBH, W, DH), _BF16),
            pltpu.VMEM((NBH, W, DH), _BF16),
            pltpu.VMEM(A_wq.shape, _BF16),
            pltpu.VMEM(A_wo.shape, _BF16),
            pltpu.VMEM(B_w1.shape, _BF16),
            pltpu.VMEM(B_w2.shape, _BF16),
            pltpu.VMEM(A_wq.shape, _BF16),
            pltpu.VMEM(A_wo.shape, _BF16),
            pltpu.VMEM(B_w1.shape, _BF16),
            pltpu.VMEM(B_w2.shape, _BF16),
            pltpu.VMEM((NBH, NJ - 1, 2, _ZC, _TILE, DH), _BF16),
            pltpu.VMEM((NBH, 2 * REP, DH), _F32),
            pltpu.VMEM((NBH, 2 * REP, DH), _F32),
            pltpu.VMEM((NBH, 2 * REP, DH), _F32),
            pltpu.VMEM((NBH, 2 * REP, DH), _F32),
            pltpu.VMEM((NBH, 2 * REP, W), _F32),
            pltpu.VMEM((NBH, 2 * REP, W), _F32),
            pltpu.VMEM((8, HQ * DH), _F32),
            pltpu.VMEM((B, D), _BF16),
            pltpu.VMEM((B, D), _BF16),
            pltpu.VMEM((F,), _BF16),
            pltpu.VMEM((D,), _BF16),
            pltpu.VMEM((B, D), _BF16),
            pltpu.VMEM((B, D), _BF16),
            pltpu.VMEM((F,), _BF16),
            pltpu.VMEM((D,), _BF16),
            pltpu.SemaphoreType.DMA((NBH,)),
            pltpu.SemaphoreType.DMA((NBH,)),
            pltpu.SemaphoreType.DMA((4,)),
            pltpu.SemaphoreType.DMA((1,)),
            pltpu.SemaphoreType.DMA((1,)),
            pltpu.SemaphoreType.DMA((4,)),
        ],
        compiler_params=pltpu.CompilerParams(vmem_limit_bytes=110 * 1024 * 1024),
    )(A_x.reshape(B, D), grad_out.reshape(B, D), B_b1, B_b2, A_k_cache, A_v_cache, A_wq, A_wo,
      B_w1, B_w2)
    return (outs[0].reshape(B, SQ, D), outs[1].reshape(B, SQ, D),
            outs[2].reshape(A_k_cache.shape), outs[3].reshape(A_v_cache.shape)) + tuple(outs[4:])
```
